```python
import jax
import jax.numpy as jnp

def _softmax(x, axis=-1):
    return jax.nn.softmax(x, axis=axis)
def _gelu(x):
    return jax.nn.gelu(x, approximate=True)
def _silu(x):
    return jax.nn.silu(x)
def _sigmoid(x):
    return jax.nn.sigmoid(x)
def _layernorm(x, axis=-1, eps=1e-5):
    m = jnp.mean(x, axis=axis, keepdims=True)
    v = jnp.var(x, axis=axis, keepdims=True)
    return (x - m) / jnp.sqrt(v + eps)
def _scatter_add(tgt, idx, src, axis=0):
    return tgt.at[idx].add(src)
def _segment_sum(src, seg, n):
    return jax.ops.segment_sum(src, seg, n)
class _Rng:
    def __init__(self, key):
        self._k = key
    def _next(self):
        self._k, sub = jax.random.split(self._k)
        return sub
    def normal(self, shape):
        return jax.random.normal(self._next(), shape, dtype=jnp.bfloat16)
    def randint(self, lo, hi, shape):
        return jax.random.randint(self._next(), shape, lo, hi, dtype=jnp.int32)
    def uniform(self, shape, lo=0.0, hi=1.0):
        return jax.random.uniform(self._next(), shape, jnp.bfloat16, lo, hi)
    def permutation(self, n):
        return jax.random.permutation(self._next(), n)


kernel_name = 'recurrent_scan__sliding_block_cached__glu_gated_swiglu__decode'

def setup_inputs():
    _rng = _Rng(jax.random.key(int.from_bytes(__import__("os").urandom(4), "little")))
    _w = (lambda a: (lambda t: t.astype(jnp.bfloat16) if jnp.issubdtype(t.dtype, jnp.floating) else t)(jnp.asarray(a)))
    def _A_setup():
        B, Sq, D = 1, 1, 640
        Hq, Hkv, Sk, Dh = 32, 32, 32768, 192
        assert Hq % Hkv == 0, (Hq, Hkv)
        return {
            "x": _w((lambda *s: _rng.normal(s) * 0.05)(B, Sq, D)),
            "k_cache": _w((lambda *s: _rng.normal(s) * 0.05)(B, Hkv, Sk, Dh)),
            "v_cache": _w((lambda *s: _rng.normal(s) * 0.05)(B, Hkv, Sk, Dh)),
            "wq": _w((lambda *s: _rng.normal(s) * 0.05)(D, Hq * Dh) * (D ** -0.5)),
            "wo": _w((lambda *s: _rng.normal(s) * 0.05)(Hq * Dh, D) * ((Hq * Dh) ** -0.5)),
        }
    _A_in = _A_setup()

    def _B_setup():
        B, S, D, F = 1, 1, 640, 1536
        return {
            "x": _w((lambda *s: _rng.normal(s) * 0.05)(B, S, D)),
            "w1": _w((lambda *s: _rng.normal(s) * 0.05)(D, F) * (2.0 / D) ** 0.5),
            "w3": _w((lambda *s: _rng.normal(s) * 0.05)(D, F) * (2.0 / D) ** 0.5),
            "w2": _w((lambda *s: _rng.normal(s) * 0.05)(F, D) * (2.0 / F) ** 0.5),
        }
    _B_in = _B_setup()

    return {
        "A_x": _A_in["x"],
        "A_k_cache": _A_in["k_cache"],
        "A_v_cache": _A_in["v_cache"],
        "A_wq": _A_in["wq"],
        "A_wo": _A_in["wo"],
        "B_x": _B_in["x"],
        "B_w1": _B_in["w1"],
        "B_w3": _B_in["w3"],
        "B_w2": _B_in["w2"],
    }

def reference(A_x, A_k_cache, A_v_cache, A_wq, A_wo, B_x, B_w1, B_w3, B_w2):
    def _A_ref(x, k_cache, v_cache, wq, wo):
        B, Sq, D = x.shape
        Hq, Dh = 32, 192
        Hkv, Sk = k_cache.shape[1], k_cache.shape[2]
        W = min(4096, max(256, Sk // 4))
        rep = Hq // Hkv
        q = (lambda x, *d: x.transpose(*d))((x @ wq).reshape(B, Sq, Hq, Dh), 0, 2, 1, 3)
        k = jnp.repeat(k_cache[:, :, Sk - W:, :], rep, axis=1)
        v = jnp.repeat(v_cache[:, :, Sk - W:, :], rep, axis=1)
        scores = jnp.einsum("bhqd,bhkd->bhqk", q, k) * (Dh ** -0.5)
        p = _softmax(scores, axis=-1)
        o = jnp.einsum("bhqk,bhkd->bhqd", p, v)
        return (lambda x, *d: x.transpose(*d))(o, 0, 2, 1, 3).reshape(B, Sq, Hq * Dh) @ wo

    def _B_ref(x, w1, w3, w2):
        gate = jnp.einsum("bsd,df->bsf", x, w1)
        up = jnp.einsum("bsd,df->bsf", x, w3)
        h = _silu(gate) * up
        out = jnp.einsum("bsf,fd->bsd", h, w2)
        return out

    x = A_x
    xn = _layernorm(x, axis=-1)
    s = _A_ref(xn, A_k_cache, A_v_cache, A_wq, A_wo)
    g = _silu(_B_ref(xn, B_w1, B_w3, B_w2))
    return x + s * g
```

```python
import functools
import numpy as np
import jax
import jax.numpy as jnp
from jax import lax
import jax.experimental.pallas as pl
import jax.experimental.pallas.tpu as pltpu

HQ, DH = 32, 192
PAIR = 2 * DH
NPAIR = HQ // 2
M = 8


def _silu(x):
    return x * jax.nn.sigmoid(x)


def build(nbuf=4, tn=4096, wo_chunks=(1536, 1536, 1024, 768, 512, 384, 256, 128), M=8):
    def kernel(x_hbm, kt_hbm, vt_hbm, wq_hbm, wo_hbm, w1_hbm, w3_hbm, w2_hbm, out_ref,
               x_v, wq_v, wo_v, w1_v, w3_v, w2_v, kbuf, vbuf, qbd, o_s, w_sem, k_sem, v_sem, wo_sem):
        D = x_v.shape[-1]
        W = kbuf.shape[-1]
        Sk = kt_hbm.shape[-1]

        def k_copy(p, slot):
            return pltpu.make_async_copy(
                kt_hbm.at[pl.ds(pl.multiple_of(p * PAIR, PAIR), PAIR), pl.ds(Sk - W, W)], kbuf.at[slot], k_sem.at[slot])

        def v_copy(p, slot):
            return pltpu.make_async_copy(
                vt_hbm.at[pl.ds(pl.multiple_of(p * PAIR, PAIR), PAIR), pl.ds(Sk - W, W)], vbuf.at[slot], v_sem.at[slot])

        offs = np.concatenate([[0], np.cumsum(wo_chunks)]).tolist()

        def wo_copy(c):
            return pltpu.make_async_copy(
                wo_hbm.at[pl.ds(offs[c], wo_chunks[c])], wo_v.at[pl.ds(offs[c], wo_chunks[c])], wo_sem.at[c])

        x_cp = pltpu.make_async_copy(x_hbm, x_v, w_sem.at[0])
        wq_cp = pltpu.make_async_copy(wq_hbm, wq_v, w_sem.at[1])
        w1_cp = pltpu.make_async_copy(w1_hbm, w1_v, w_sem.at[2])
        w3_cp = pltpu.make_async_copy(w3_hbm, w3_v, w_sem.at[3])
        w2_cp = pltpu.make_async_copy(w2_hbm, w2_v, w_sem.at[4])

        x_cp.start()
        wq_cp.start()
        w1_cp.start()
        w3_cp.start()
        w2_cp.start()
        for p in range(nbuf):
            k_copy(p, p).start()
            v_copy(p, p).start()

        x_cp.wait()
        x = x_v[0].astype(jnp.float32)
        mean = jnp.mean(x, axis=-1, keepdims=True)
        xc = x - mean
        var = jnp.mean(xc * xc, axis=-1, keepdims=True)
        xn = xc / jnp.sqrt(var + 1e-5)
        xn = jnp.broadcast_to(xn, (M, D)).astype(jnp.bfloat16)

        row = lax.broadcasted_iota(jnp.int32, (M, PAIR), 0)
        col = lax.broadcasted_iota(jnp.int32, (M, PAIR), 1)
        own = ((row == 0) & (col < DH)) | ((row == 1) & (col >= DH))

        wq_cp.wait()

        def q_body(p, c):
            w = wq_v[:, pl.ds(pl.multiple_of(p * PAIR, 128), PAIR)]
            q = jnp.dot(xn, w, preferred_element_type=jnp.float32)
            qbd[p] = jnp.where(own, q, 0.0)
            return c
        lax.fori_loop(0, NPAIR, q_body, 0)

        w1_cp.wait()
        gate = jnp.dot(xn, w1_v[...], preferred_element_type=jnp.float32)
        w3_cp.wait()
        up = jnp.dot(xn, w3_v[...], preferred_element_type=jnp.float32)
        h = (_silu(gate) * up).astype(jnp.bfloat16)
        w2_cp.wait()
        g = _silu(jnp.dot(h, w2_v[...], preferred_element_type=jnp.float32))

        scale = DH ** -0.5

        def pair_body(p, c):
            slot = lax.rem(p, nbuf)
            k_copy(p, slot).wait()
            q = qbd[p].astype(jnp.bfloat16)
            s = jnp.dot(q, kbuf[slot], preferred_element_type=jnp.float32) * scale

            @pl.when(p + nbuf < NPAIR)
            def _():
                k_copy(p + nbuf, slot).start()

            m = jnp.max(s, axis=-1, keepdims=True)
            e = jnp.exp(s - m)
            l = jnp.sum(e, axis=-1, keepdims=True)
            v_copy(p, slot).wait()
            o = lax.dot_general(e.astype(jnp.bfloat16), vbuf[slot], (((1,), (1,)), ((), ())),
                                preferred_element_type=jnp.float32)

            @pl.when(p + nbuf < NPAIR)
            def _():
                v_copy(p + nbuf, slot).start()

            @pl.when(p + nbuf == NPAIR - 1)
            def _():
                for cidx in range(len(wo_chunks)):
                    wo_copy(cidx).start()

            o = jnp.where(own, o / l, 0.0)
            o_s[:, pl.ds(pl.multiple_of(p * PAIR, 128), PAIR)] = o
            return c
        lax.fori_loop(0, NPAIR, pair_body, 0)

        acc = jnp.zeros((M, D), jnp.float32)
        for cidx in range(len(wo_chunks)):
            wo_copy(cidx).wait()
            lo, n = offs[cidx], wo_chunks[cidx]
            acc = acc + jnp.dot(o_s[:, lo:lo + n].astype(jnp.bfloat16), wo_v[lo:lo + n, :],
                                preferred_element_type=jnp.float32)
        s_out = jnp.sum(acc, axis=0, keepdims=True)
        out_ref[0] = (x + s_out * g[0:1]).astype(out_ref.dtype)

    def fn(A_x, A_k_cache, A_v_cache, A_wq, A_wo, B_x, B_w1, B_w3, B_w2):
        B, Sq, D = A_x.shape
        _, Hkv, Sk, Dh = A_k_cache.shape
        W = min(4096, max(256, Sk // 4))
        F = B_w1.shape[1]
        kt = jnp.swapaxes(A_k_cache, 2, 3).reshape(Hkv * Dh, Sk)
        vt = jnp.swapaxes(A_v_cache, 2, 3).reshape(Hkv * Dh, Sk)
        hbm = pl.BlockSpec(memory_space=pltpu.HBM)
        dt = A_x.dtype
        return pl.pallas_call(
            kernel,
            out_shape=jax.ShapeDtypeStruct((B, Sq, D), dt),
            in_specs=[hbm] * 8,
            out_specs=pl.BlockSpec(memory_space=pltpu.VMEM),
            scratch_shapes=[
                pltpu.VMEM((B, Sq, D), dt),
                pltpu.VMEM(A_wq.shape, dt),
                pltpu.VMEM(A_wo.shape, dt),
                pltpu.VMEM(B_w1.shape, dt),
                pltpu.VMEM(B_w3.shape, dt),
                pltpu.VMEM(B_w2.shape, dt),
                pltpu.VMEM((nbuf, PAIR, W), dt),
                pltpu.VMEM((nbuf, PAIR, W), dt),
                pltpu.VMEM((NPAIR, M, PAIR), jnp.float32),
                pltpu.VMEM((M, HQ * DH), jnp.float32),
                pltpu.SemaphoreType.DMA((5,)),
                pltpu.SemaphoreType.DMA((nbuf,)),
                pltpu.SemaphoreType.DMA((nbuf,)),
                pltpu.SemaphoreType.DMA((len(wo_chunks),)),
            ],
            compiler_params=pltpu.CompilerParams(vmem_limit_bytes=110 * 1024 * 1024),
        )(A_x, kt, vt, A_wq, A_wo, B_w1, B_w3, B_w2)
    return fn


_impl = build()


@jax.jit
def pallas_recurrent_scan__sliding_block_cached__glu_gated_swiglu__decode_kernel(
    A_x: jax.Array,
    A_k_cache: jax.Array,
    A_v_cache: jax.Array,
    A_wq: jax.Array,
    A_wo: jax.Array,
    B_x: jax.Array,
    B_w1: jax.Array,
    B_w3: jax.Array,
    B_w2: jax.Array,
):
    return _impl(A_x, A_k_cache, A_v_cache, A_wq, A_wo, B_x, B_w1, B_w3, B_w2)
```

```python
import numpy as np
import jax
import jax.numpy as jnp
from jax import lax
import jax.experimental.pallas as pl
import jax.experimental.pallas.tpu as pltpu

HQ, DH = 32, 192
PAIR = 2 * DH
NPAIR = HQ // 2
M = 8
NBUF = 2


def _silu(x):
    return x * jax.nn.sigmoid(x)


def _tiles(R, C, r, c, pat, order="cr"):
    if order == "rc":
        subs = [(a * r, b * c) for a in range(R // r) for b in range(C // c)]
    else:
        subs = [(a * r, b * c) for b in range(C // c) for a in range(R // r)]
    return [(a, b, r, c, pat[i % len(pat)]) for i, (a, b) in enumerate(subs)]


def _split(items, n):
    cuts = [len(items) * i // n for i in range(n + 1)]
    return [items[cuts[i]:cuts[i + 1]] for i in range(n)]


def build(kv=(32, 512, (0, 1)), tn=512, wq_t=(128, 128, (0, 1)), w13_t=(128, 128, (0, 1)), w2_t=(32, 640, (0, 1, 1)),
          wo_t=(32, (0, 1, 1)), wo_tail=(768, 384, 256, 128)):
    def kernel(x_hbm, kt_hbm, vt_hbm, wq_hbm, wo_hbm, w1_hbm, w3_hbm, w2_hbm, out_ref,
               x_v, wq_v, wo_v, w1_v, w3_v, w2_v, kbuf, vbuf, qbd, o_s, w_sem, k_sem, v_sem):
        D = x_v.shape[-1]
        W = kbuf.shape[-1]
        Sk = kt_hbm.shape[-1]
        F = w1_v.shape[1]
        nblk = W // tn

        def start_w(src, dst, sem, tiles):
            for (a, b, r, c, pr) in tiles:
                pltpu.make_async_copy(src.at[pl.ds(a, r), pl.ds(b, c)], dst.at[pl.ds(a, r), pl.ds(b, c)],
                                      sem).start(priority=pr)

        def start_kv(src, dst, sem, p, slot, tiles):
            for (a, b, r, c, pr) in tiles:
                r0 = p * PAIR + a
                if not isinstance(r0, int):
                    r0 = pl.multiple_of(r0, r)
                pltpu.make_async_copy(src.at[pl.ds(r0, r), pl.ds(Sk - W + b, c)],
                                      dst.at[slot, pl.ds(a, r), pl.ds(b, c)], sem.at[slot]).start(priority=pr)

        def wait_all(dst, sem):
            pltpu.make_async_copy(dst, dst, sem).wait()

        kv_tiles = _tiles(PAIR, W, *kv)
        kv_blk = _split(kv_tiles, nblk)

        HD = HQ * DH
        quarter = HD // 4
        parts = [quarter] * 3 + list(wo_tail)
        offs = np.concatenate([[0], np.cumsum(parts)]).tolist()
        wo_r, wo_pat = wo_t
        wo_per_blk = quarter // wo_r // nblk

        def wo_sem(i):
            return w_sem.at[i]

        def part_of(row):
            return int(np.searchsorted(offs, row, side="right") - 1)

        def start_wo(p, phase, b):
            last = p == NPAIR - 1
            for i in range(wo_per_blk):
                j = b * wo_per_blk + i
                lo = phase * quarter + j * wo_r
                r0 = pl.multiple_of(jnp.where(last, lo + 2 * quarter, lo), wo_r)
                si = jnp.where(last, part_of(lo + 2 * quarter), part_of(lo))
                pltpu.make_async_copy(wo_hbm.at[pl.ds(r0, wo_r)], wo_v.at[pl.ds(r0, wo_r)],
                                      w_sem.at[si]).start(priority=wo_pat[j % len(wo_pat)])

        x_cp = pltpu.make_async_copy(x_hbm, x_v, w_sem.at[0])
        x_cp.start()
        start_w(wq_hbm, wq_v, w_sem.at[1], _tiles(D, HD, *wq_t))
        start_w(w1_hbm, w1_v, w_sem.at[2], _tiles(D, F, *w13_t))
        start_w(w3_hbm, w3_v, w_sem.at[3], _tiles(D, F, *w13_t))
        start_w(w2_hbm, w2_v, w_sem.at[4], _tiles(F, D, *w2_t))

        x_cp.wait()
        x = x_v[0].astype(jnp.float32)
        mean = jnp.mean(x, axis=-1, keepdims=True)
        xc = x - mean
        var = jnp.mean(xc * xc, axis=-1, keepdims=True)
        xn = xc / jnp.sqrt(var + 1e-5)
        xn = jnp.broadcast_to(xn, (M, D)).astype(jnp.bfloat16)

        row = lax.broadcasted_iota(jnp.int32, (M, PAIR), 0)
        col = lax.broadcasted_iota(jnp.int32, (M, PAIR), 1)
        own = ((row == 0) & (col < DH)) | ((row == 1) & (col >= DH))

        start_kv(kt_hbm, kbuf, k_sem, 0, 0, kv_tiles)
        wait_all(wq_v, w_sem.at[1])

        def q_body(p, c):
            w = wq_v[:, pl.ds(pl.multiple_of(p * PAIR, 128), PAIR)]
            q = jnp.dot(xn, w, preferred_element_type=jnp.float32)
            qbd[p] = jnp.where(own, q, 0.0)
            return c
        lax.fori_loop(0, NPAIR, q_body, 0)

        start_kv(vt_hbm, vbuf, v_sem, 0, 0, kv_tiles)
        wait_all(w1_v, w_sem.at[2])
        gate = jnp.dot(xn, w1_v[...], preferred_element_type=jnp.float32)
        wait_all(w3_v, w_sem.at[3])
        up = jnp.dot(xn, w3_v[...], preferred_element_type=jnp.float32)
        h = (_silu(gate) * up).astype(jnp.bfloat16)
        start_kv(kt_hbm, kbuf, k_sem, 1, 1, kv_tiles)
        wait_all(w2_v, w_sem.at[4])
        g = _silu(jnp.dot(h, w2_v[...], preferred_element_type=jnp.float32))
        start_kv(vt_hbm, vbuf, v_sem, 1, 1, kv_tiles)

        scale = DH ** -0.5

        def pair_body(p, c):
            slot = lax.rem(p, NBUF)
            more = p + NBUF < NPAIR

            wait_all(kbuf.at[slot], k_sem.at[slot])
            q = qbd[p].astype(jnp.bfloat16)
            s = []
            for b in range(nblk):
                s.append(jnp.dot(q, kbuf[slot, :, b * tn:(b + 1) * tn], preferred_element_type=jnp.float32) * scale)
                pl.when(more)(lambda: start_kv(kt_hbm, kbuf, k_sem, p + NBUF, slot, kv_blk[b]))
                pl.when(jnp.logical_not(more))(lambda: start_wo(p, 0, b))

            m = s[0]
            for sb in s[1:]:
                m = jnp.maximum(m, sb)
            m = jnp.max(m, axis=-1, keepdims=True)
            e = [jnp.exp(sb - m) for sb in s]
            l = e[0]
            for eb in e[1:]:
                l = l + eb
            l = jnp.sum(l, axis=-1, keepdims=True)

            wait_all(vbuf.at[slot], v_sem.at[slot])
            o = None
            for b in range(nblk):
                ob = lax.dot_general(e[b].astype(jnp.bfloat16), vbuf[slot, :, b * tn:(b + 1) * tn],
                                     (((1,), (1,)), ((), ())), preferred_element_type=jnp.float32)
                o = ob if o is None else o + ob
                pl.when(more)(lambda: start_kv(vt_hbm, vbuf, v_sem, p + NBUF, slot, kv_blk[b]))
                pl.when(jnp.logical_not(more))(lambda: start_wo(p, 1, b))

            o = jnp.where(own, o / l, 0.0)
            o_s[:, pl.ds(pl.multiple_of(p * PAIR, 128), PAIR)] = o
            return c
        lax.fori_loop(0, NPAIR, pair_body, 0)

        acc = None
        for i, n in enumerate(parts):
            lo = offs[i]
            wait_all(wo_v.at[pl.ds(lo, n)], w_sem.at[i])
            part = jnp.dot(o_s[:, lo:lo + n].astype(jnp.bfloat16), wo_v[lo:lo + n, :],
                           preferred_element_type=jnp.float32)
            acc = part if acc is None else acc + part
        s_out = acc[0:1] + acc[1:2]
        out_ref[0] = (x + s_out * g[0:1]).astype(out_ref.dtype)

    def fn(A_x, A_k_cache, A_v_cache, A_wq, A_wo, B_x, B_w1, B_w3, B_w2):
        B, Sq, D = A_x.shape
        _, Hkv, Sk, Dh = A_k_cache.shape
        W = min(4096, max(256, Sk // 4))
        kt = jnp.swapaxes(A_k_cache, 2, 3).reshape(Hkv * Dh, Sk)
        vt = jnp.swapaxes(A_v_cache, 2, 3).reshape(Hkv * Dh, Sk)
        hbm = pl.BlockSpec(memory_space=pltpu.HBM)
        dt = A_x.dtype
        return pl.pallas_call(
            kernel,
            out_shape=jax.ShapeDtypeStruct((B, Sq, D), dt),
            in_specs=[hbm] * 8,
            out_specs=pl.BlockSpec(memory_space=pltpu.VMEM),
            scratch_shapes=[
                pltpu.VMEM((B, Sq, D), dt),
                pltpu.VMEM(A_wq.shape, dt),
                pltpu.VMEM(A_wo.shape, dt),
                pltpu.VMEM(B_w1.shape, dt),
                pltpu.VMEM(B_w3.shape, dt),
                pltpu.VMEM(B_w2.shape, dt),
                pltpu.VMEM((NBUF, PAIR, W), dt),
                pltpu.VMEM((NBUF, PAIR, W), dt),
                pltpu.VMEM((NPAIR, M, PAIR), jnp.float32),
                pltpu.VMEM((M, HQ * DH), jnp.float32),
                pltpu.SemaphoreType.DMA((max(5, 3 + len(wo_tail)),)),
                pltpu.SemaphoreType.DMA((NBUF,)),
                pltpu.SemaphoreType.DMA((NBUF,)),
            ],
            compiler_params=pltpu.CompilerParams(vmem_limit_bytes=110 * 1024 * 1024),
        )(A_x, kt, vt, A_wq, A_wo, B_w1, B_w3, B_w2)
    return fn


_impl = build(kv=(32, 512, (0, 1, 1)))


@jax.jit
def pallas_recurrent_scan__sliding_block_cached__glu_gated_swiglu__decode_kernel(
    A_x: jax.Array,
    A_k_cache: jax.Array,
    A_v_cache: jax.Array,
    A_wq: jax.Array,
    A_wo: jax.Array,
    B_x: jax.Array,
    B_w1: jax.Array,
    B_w3: jax.Array,
    B_w2: jax.Array,
):
    return _impl(A_x, A_k_cache, A_v_cache, A_wq, A_wo, B_x, B_w1, B_w3, B_w2)
```

```python
import numpy as np
import jax
import jax.numpy as jnp
from jax import lax
import jax.experimental.pallas as pl
import jax.experimental.pallas.tpu as pltpu

HQ, DH = 32, 192
PAIR = 2 * DH
NPAIR = HQ // 2
M = 8
NBUF = 2
WQ_SLABS = 5
WO_SLABS = 12


def _silu(x):
    return x * jax.nn.sigmoid(x)


def _grid(R, C, r, c, order="cr"):
    if order == "rc":
        return [(a * r, b * c) for a in range(R // r) for b in range(C // c)]
    return [(a * r, b * c) for b in range(C // c) for a in range(R // r)]


def _split(items, n):
    cuts = [len(items) * i // n for i in range(n + 1)]
    return [items[cuts[i]:cuts[i + 1]] for i in range(n)]


def build(kv=(32, 512, (0, 1, 1)), tn=512, wq_t=(5, 8, 512, (0, 1, 1)), wo_g=4, wo_pat=(0, 1, 1),
          ffn_t=(40, 512, 32, (0, 1, 1)), wo_tail=(1024, 512, 256, 128, 128), lead=0, nobc=False, nosc=False):
    def kernel(x_hbm, kt_hbm, vt_hbm, wq_hbm, wo_hbm, w1_hbm, w3_hbm, w2_hbm, out_ref,
               x_v, wq_v, wo_v, w1_v, w3_v, w2_v, kbuf, vbuf, qbd, o_s, acc_s, w_sem, k_sem, v_sem):
        D = x_v.shape[-1]
        W = kbuf.shape[-1]
        Sk = kt_hbm.shape[-1]
        F = w1_v.shape[1]
        HD = HQ * DH
        nblk = W // tn
        kr, kc, kpat = kv

        def mult(i, n):
            return i if isinstance(i, int) else pl.multiple_of(i, n)

        def wait_all(dst, sem):
            pltpu.make_async_copy(dst, dst, sem).wait()

        kv_tiles = [(a, b, kpat[i % len(kpat)]) for i, (a, b) in enumerate(_grid(PAIR, W, kr, kc))]
        kv_blk = _split(kv_tiles, nblk)

        def start_kv(src, dst, sem, p, slot, tiles):
            for (a, b, pr) in tiles:
                pltpu.make_async_copy(src.at[pl.ds(mult(p * PAIR + a, kr), kr), pl.ds(mult(Sk - W + b, kc), kc)],
                                      dst.at[slot, pl.ds(mult(a, kr), kr), pl.ds(mult(b, kc), kc)],
                                      sem.at[slot]).start(priority=pr)

        wo_rows = HD // WO_SLABS
        tail_rows = sum(wo_tail)
        head_slabs = (HD - tail_rows) // wo_rows
        tail_offs = (HD - tail_rows + np.concatenate([[0], np.cumsum(wo_tail)])).tolist()
        wo_plan = []
        for s in range(0, head_slabs, wo_g):
            for a in range(0, wo_rows, 8):
                wo_plan.append((s, wo_g, a, 8, 0))
        for r0 in range(HD - tail_rows, HD, 32):
            wo_plan.append((r0 // wo_rows, 1, r0 % wo_rows, 32, int(np.searchsorted(tail_offs, r0, side="right"))))
        wo_plan = [t + (wo_pat[i % len(wo_pat)],) for i, t in enumerate(wo_plan)]
        wo_blk = _split(wo_plan, 4 * nblk)

        def start_wo(i):
            for (s, g, a, r, si, pr) in wo_blk[i]:
                pltpu.make_async_copy(wo_hbm.at[pl.ds(s, g), pl.ds(a, r)], wo_v.at[pl.ds(s, g), pl.ds(a, r)],
                                      w_sem.at[si]).start(priority=pr)

        x_cp = pltpu.make_async_copy(x_hbm, x_v, w_sem.at[0])
        x_cp.start()
        qg, qr, qc, qpat = wq_t
        i = 0
        for (a, b) in _grid(D // WQ_SLABS, HD, qr, qc, "rc"):
            for s in range(0, WQ_SLABS, qg):
                pltpu.make_async_copy(wq_hbm.at[pl.ds(s, qg), pl.ds(a, qr), pl.ds(b, qc)],
                                      wq_v.at[pl.ds(s, qg), pl.ds(a, qr), pl.ds(b, qc)],
                                      w_sem.at[1]).start(priority=1 if i < lead else qpat[i % len(qpat)])
                i += 1
        fr, fc, f2r, fpat = ffn_t
        up_tiles = _grid(D, F, fr, fc)
        dn_tiles = _split(list(range(0, F, f2r)), len(up_tiles))
        i = 0
        for (a, b), dn in zip(up_tiles, dn_tiles):
            for src, dst in ((w1_hbm, w1_v), (w3_hbm, w3_v)):
                pltpu.make_async_copy(src.at[pl.ds(a, fr), pl.ds(b, fc)], dst.at[pl.ds(a, fr), pl.ds(b, fc)],
                                      w_sem.at[2]).start(priority=fpat[i % len(fpat)])
                i += 1
            for a2 in dn:
                pltpu.make_async_copy(w2_hbm.at[pl.ds(a2, f2r)], w2_v.at[pl.ds(a2, f2r)],
                                      w_sem.at[2]).start(priority=fpat[i % len(fpat)])
                i += 1

        x_cp.wait()
        x = x_v[0].astype(jnp.float32)
        mean = jnp.mean(x, axis=-1, keepdims=True)
        xc = x - mean
        var = jnp.mean(xc * xc, axis=-1, keepdims=True)
        xn = xc / jnp.sqrt(var + 1e-5)
        xn = jnp.broadcast_to(xn, (M, D)).astype(jnp.bfloat16)

        row = lax.broadcasted_iota(jnp.int32, (M, PAIR), 0)
        col = lax.broadcasted_iota(jnp.int32, (M, PAIR), 1)
        own = ((row == 0) & (col < DH)) | ((row == 1) & (col >= DH))

        wait_all(wq_v, w_sem.at[1])
        per = NPAIR // nblk

        def q_body(b, c):
            for j in range(per):
                p = b * per + j
                w = wq_v[:, :, pl.ds(pl.multiple_of(p * PAIR, 128), PAIR)].reshape(D, PAIR)
                qbd[p] = jnp.where(own, jnp.dot(xn, w, preferred_element_type=jnp.float32), 0.0)
            start_kv(kt_hbm, kbuf, k_sem, 0, 0, [(a, b * tn + bb, pr) for (a, bb, pr) in kv_blk[0]])
            return c
        lax.fori_loop(0, nblk, q_body, 0)

        start_kv(vt_hbm, vbuf, v_sem, 0, 0, kv_tiles)
        wait_all(w1_v, w_sem.at[2])
        wait_all(w3_v, w_sem.at[2])
        wait_all(w2_v, w_sem.at[2])
        gate = jnp.dot(xn, w1_v[...], preferred_element_type=jnp.float32)
        up = jnp.dot(xn, w3_v[...], preferred_element_type=jnp.float32)
        h = (_silu(gate) * up).astype(jnp.bfloat16)
        start_kv(kt_hbm, kbuf, k_sem, 1, 1, kv_tiles)
        g = _silu(jnp.dot(h, w2_v[...], preferred_element_type=jnp.float32))
        start_kv(vt_hbm, vbuf, v_sem, 1, 1, kv_tiles)

        scale = DH ** -0.5

        def pair_body(p, c):
            slot = lax.rem(p, NBUF)

            def refill(src, dst, sem, phase, b):
                pl.when(p < NPAIR - 2)(lambda: start_kv(src, dst, sem, p + NBUF, slot, kv_blk[b]))
                pl.when(p == NPAIR - 2)(lambda: start_wo(phase * nblk + b))
                pl.when(p == NPAIR - 1)(lambda: start_wo((2 + phase) * nblk + b))

            wait_all(kbuf.at[slot], k_sem.at[slot])
            q = qbd[p].astype(jnp.bfloat16)
            s = []
            for b in range(nblk):
                s.append(jnp.dot(q, kbuf[slot, :, b * tn:(b + 1) * tn], preferred_element_type=jnp.float32) * scale)
                refill(kt_hbm, kbuf, k_sem, 0, b)

            m = s[0]
            for sb in s[1:]:
                m = jnp.maximum(m, sb)
            m = jnp.max(m, axis=-1, keepdims=True)
            e = [jnp.exp(sb - m) for sb in s]
            l = e[0]
            for eb in e[1:]:
                l = l + eb
            l = jnp.sum(l, axis=-1, keepdims=True)

            wait_all(vbuf.at[slot], v_sem.at[slot])
            o = None
            for b in range(nblk):
                ob = lax.dot_general(e[b].astype(jnp.bfloat16), vbuf[slot, :, b * tn:(b + 1) * tn],
                                     (((1,), (1,)), ((), ())), preferred_element_type=jnp.float32)
                o = ob if o is None else o + ob
                refill(vt_hbm, vbuf, v_sem, 1, b)

            o = jnp.where(own, o / l, 0.0)
            o_s[:, pl.ds(pl.multiple_of(p * PAIR, 128), PAIR)] = o
            return c
        lax.fori_loop(0, NPAIR, pair_body, 0)

        def wo_rows_dot(lo, n):
            s0, a0 = lo // wo_rows, lo % wo_rows
            if n >= wo_rows:
                w = wo_v[s0:s0 + n // wo_rows].reshape(n, D)
            else:
                w = wo_v[s0, a0:a0 + n]
            return jnp.dot(o_s[:, lo:lo + n].astype(jnp.bfloat16), w, preferred_element_type=jnp.float32)

        def wo_rows_ref(lo, n):
            s0, a0 = lo // wo_rows, lo % wo_rows
            return wo_v.at[pl.ds(s0, n // wo_rows)] if n >= wo_rows else wo_v.at[s0, pl.ds(a0, n)]

        wait_all(wo_rows_ref(0, HD - tail_rows), w_sem.at[0])
        acc_s[...] = wo_rows_dot(0, HD - tail_rows)
        for i, n in enumerate(wo_tail):
            lo = tail_offs[i]
            wait_all(wo_rows_ref(lo, n), w_sem.at[i + 1])
            if i < len(wo_tail) - 1:
                acc_s[...] += wo_rows_dot(lo, n)
            else:
                acc = acc_s[...] + wo_rows_dot(lo, n)
        s_out = acc[0:1] + acc[1:2]
        out_ref[0] = (x + s_out * g[0:1]).astype(out_ref.dtype)

    def fn(A_x, A_k_cache, A_v_cache, A_wq, A_wo, B_x, B_w1, B_w3, B_w2):
        B, Sq, D = A_x.shape
        _, Hkv, Sk, Dh = A_k_cache.shape
        W = min(4096, max(256, Sk // 4))
        kt = jnp.swapaxes(A_k_cache, 2, 3).reshape(Hkv * Dh, Sk)
        vt = jnp.swapaxes(A_v_cache, 2, 3).reshape(Hkv * Dh, Sk)
        wq3 = A_wq.reshape(WQ_SLABS, D // WQ_SLABS, HQ * DH)
        wo3 = A_wo.reshape(WO_SLABS, HQ * DH // WO_SLABS, D)
        hbm = pl.BlockSpec(memory_space=pltpu.HBM)
        dt = A_x.dtype
        return pl.pallas_call(
            kernel,
            out_shape=jax.ShapeDtypeStruct((B, Sq, D), dt),
            in_specs=[hbm] * 8,
            out_specs=pl.BlockSpec(memory_space=pltpu.VMEM),
            scratch_shapes=[
                pltpu.VMEM((B, Sq, D), dt),
                pltpu.VMEM(wq3.shape, dt),
                pltpu.VMEM(wo3.shape, dt),
                pltpu.VMEM(B_w1.shape, dt),
                pltpu.VMEM(B_w3.shape, dt),
                pltpu.VMEM(B_w2.shape, dt),
                pltpu.VMEM((NBUF, PAIR, W), dt),
                pltpu.VMEM((NBUF, PAIR, W), dt),
                pltpu.VMEM((NPAIR, M, PAIR), jnp.float32),
                pltpu.VMEM((M, HQ * DH), jnp.float32),
                pltpu.VMEM((M, D), jnp.float32),
                pltpu.SemaphoreType.DMA((max(3, 1 + len(wo_tail)),)),
                pltpu.SemaphoreType.DMA((NBUF,)),
                pltpu.SemaphoreType.DMA((NBUF,)),
            ],
            compiler_params=pltpu.CompilerParams(vmem_limit_bytes=110 * 1024 * 1024, disable_bounds_checks=nobc, disable_semaphore_checks=nosc),
        )(A_x, kt, vt, wq3, wo3, B_w1, B_w3, B_w2)
    return fn


_impl = build(kv=(16, 512, (0, 1, 1, 1)))


@jax.jit
def pallas_recurrent_scan__sliding_block_cached__glu_gated_swiglu__decode_kernel(
    A_x: jax.Array,
    A_k_cache: jax.Array,
    A_v_cache: jax.Array,
    A_wq: jax.Array,
    A_wo: jax.Array,
    B_x: jax.Array,
    B_w1: jax.Array,
    B_w3: jax.Array,
    B_w2: jax.Array,
):
    return _impl(A_x, A_k_cache, A_v_cache, A_wq, A_wo, B_x, B_w1, B_w3, B_w2)
```

```python
import numpy as np
import jax
import jax.numpy as jnp
from jax import lax
import jax.experimental.pallas as pl
import jax.experimental.pallas.tpu as pltpu

HQ, DH = 32, 192
PAIR = 2 * DH
NPAIR = HQ // 2
M = 8
NBUF = 2


def _silu(x):
    return x * jax.nn.sigmoid(x)


def _split(items, n):
    cuts = [len(items) * i // n for i in range(n + 1)]
    return [items[cuts[i]:cuts[i + 1]] for i in range(n)]


def _strided(lo, hi, step, slabs):
    h = (hi - lo) // slabs
    assert h * slabs == hi - lo and h % step == 0
    return [lo + s * h + a for a in range(0, h, step) for s in range(slabs)]


def build(tn=2048, wq_slabs=20, wo_r=24, wo_slabs=8, wo_tr=32, up_slabs=1, dn_slabs=1, wo_tail=(2048, 768, 256),
          tail_p1=0):
    def kernel(x_hbm, kt_hbm, vt_hbm, wq_hbm, wo_hbm, w1_hbm, w3_hbm, w2_hbm, out_ref,
               x_v, wq_v, wo_v, w1_v, w3_v, w2_v, kbuf, vbuf, qbd, o_s, acc_s, sems):
        D = x_v.shape[-1]
        W = kbuf.shape[-1]
        Sk = kt_hbm.shape[-1]
        F = w1_v.shape[1]
        HD = HQ * DH
        nblk = W // tn

        def mult(i, n):
            return i if isinstance(i, int) else pl.multiple_of(i, n)

        def wait_all(dst, sem):
            pltpu.make_async_copy(dst, dst, sem).wait()

        def k_sem(slot):
            return sems.at[2 * slot]

        def v_sem(slot):
            return sems.at[2 * slot + 1]

        def start_w(src, dst, sem, r0, r, c0, c, prio):
            pltpu.make_async_copy(src.at[pl.ds(r0, r), pl.ds(c0, c)], dst.at[pl.ds(r0, r), pl.ds(c0, c)],
                                  sem).start(priority=prio)

        def start_kv(src, dst, sem, p, slot, b, rows=range(0, PAIR, 8)):
            for i, a in enumerate(rows):
                pltpu.make_async_copy(src.at[pl.ds(mult(p * PAIR + a, 8), 8), pl.ds(mult(Sk - W + b * tn, tn), tn)],
                                      dst.at[slot, pl.ds(mult(a, 8), 8), pl.ds(mult(b * tn, tn), tn)],
                                      sem).start(priority=i % 2)

        head_rows = HD - sum(wo_tail)
        tail_offs = (head_rows + np.concatenate([[0], np.cumsum(wo_tail)])).tolist()
        head = [(r0, wo_r, 0) for r0 in _strided(0, head_rows, wo_r, wo_slabs)]
        tail = [(r0, wo_tr, int(np.searchsorted(tail_offs, r0, side="right"))) for r0 in range(head_rows, HD, wo_tr)]
        plan = [t + (1 if t[0] >= HD - tail_p1 else i % 2,) for i, t in enumerate(head + tail)]
        nh = 4 * nblk * head_rows // HD
        wo_blk = _split(plan[:len(head)], nh) + _split(plan[len(head):], 4 * nblk - nh)
        for i, blk in enumerate(wo_blk):
            assert all(i >= t[2] * nblk for t in blk), i

        def start_wo(i):
            for (r0, r, si, pr) in wo_blk[i]:
                start_w(wo_hbm, wo_v, sems.at[si], r0, r, 0, D, pr)

        x_cp = pltpu.make_async_copy(x_hbm, x_v, v_sem(1))
        x_cp.start()
        for i, (a, b) in enumerate([(a, b) for a0 in range(0, D // wq_slabs, 8) for b in range(0, HD, 2048)
                                    for a in range(a0, D, D // wq_slabs)]):
            start_w(wq_hbm, wq_v, k_sem(1), a, 8, b, 2048, (i + 1) % 2)
        x_cp.wait()
        up_rows, dn_rows = _strided(0, D, 8, up_slabs), _strided(0, F, 24, dn_slabs)
        ffn = []
        for a, dn in zip(up_rows, _split(dn_rows, len(up_rows))):
            ffn += [(w1_hbm, w1_v, a, 8, F), (w3_hbm, w3_v, a, 8, F)] + [(w2_hbm, w2_v, a2, 24, D) for a2 in dn]
        for i, (src, dst, a, r, c) in enumerate(ffn):
            start_w(src, dst, v_sem(1), a, r, 0, c, (i + 1) % 2)

        x = x_v[0].astype(jnp.float32)
        mean = jnp.mean(x, axis=-1, keepdims=True)
        xc = x - mean
        var = jnp.mean(xc * xc, axis=-1, keepdims=True)
        xn = xc / jnp.sqrt(var + 1e-5)
        xn = jnp.broadcast_to(xn, (M, D)).astype(jnp.bfloat16)

        row = lax.broadcasted_iota(jnp.int32, (M, PAIR), 0)
        col = lax.broadcasted_iota(jnp.int32, (M, PAIR), 1)
        own = ((row == 0) & (col < DH)) | ((row == 1) & (col >= DH))

        wait_all(wq_v, k_sem(1))
        per = PAIR * nblk // NPAIR

        def q_body(p, c):
            w = wq_v[:, pl.ds(pl.multiple_of(p * PAIR, 128), PAIR)]
            qbd[p] = jnp.where(own, jnp.dot(xn, w, preferred_element_type=jnp.float32), 0.0)
            b, a0 = lax.div(p * per, PAIR), lax.rem(p * per, PAIR)
            start_kv(kt_hbm, kbuf, k_sem(0), 0, 0, b, [a0 + a for a in range(0, per, 8)])
            return c
        lax.fori_loop(0, NPAIR, q_body, 0)

        for b in range(nblk):
            start_kv(vt_hbm, vbuf, v_sem(0), 0, 0, b)
        wait_all(w1_v, v_sem(1))
        wait_all(w3_v, v_sem(1))
        wait_all(w2_v, v_sem(1))
        gate = jnp.dot(xn, w1_v[...], preferred_element_type=jnp.float32)
        up = jnp.dot(xn, w3_v[...], preferred_element_type=jnp.float32)
        h = (_silu(gate) * up).astype(jnp.bfloat16)
        for b in range(nblk):
            start_kv(kt_hbm, kbuf, k_sem(1), 1, 1, b)
        g = _silu(jnp.dot(h, w2_v[...], preferred_element_type=jnp.float32))
        for b in range(nblk):
            start_kv(vt_hbm, vbuf, v_sem(1), 1, 1, b)

        scale = DH ** -0.5

        def pair_body(p, c):
            slot = lax.rem(p, NBUF)

            def refill(src, dst, sem, phase, b):
                pl.when(p < NPAIR - 2)(lambda: start_kv(src, dst, sem, p + NBUF, slot, b))
                pl.when(p == NPAIR - 2)(lambda: start_wo(phase * nblk + b))
                pl.when(p == NPAIR - 1)(lambda: start_wo((2 + phase) * nblk + b))

            wait_all(kbuf.at[slot], k_sem(slot))
            q = qbd[p].astype(jnp.bfloat16)
            s = []
            for b in range(nblk):
                s.append(jnp.dot(q, kbuf[slot, :, b * tn:(b + 1) * tn], preferred_element_type=jnp.float32) * scale)
                refill(kt_hbm, kbuf, k_sem(slot), 0, b)

            m = s[0]
            for sb in s[1:]:
                m = jnp.maximum(m, sb)
            m = jnp.max(m, axis=-1, keepdims=True)
            e = [jnp.exp(sb - m) for sb in s]
            l = e[0]
            for eb in e[1:]:
                l = l + eb
            l = jnp.sum(l, axis=-1, keepdims=True)

            wait_all(vbuf.at[slot], v_sem(slot))
            o = None
            for b in range(nblk):
                ob = lax.dot_general(e[b].astype(jnp.bfloat16), vbuf[slot, :, b * tn:(b + 1) * tn],
                                     (((1,), (1,)), ((), ())), preferred_element_type=jnp.float32)
                o = ob if o is None else o + ob
                refill(vt_hbm, vbuf, v_sem(slot), 1, b)

            o = jnp.where(own, o / l, 0.0)
            o_s[:, pl.ds(pl.multiple_of(p * PAIR, 128), PAIR)] = o
            return c
        lax.fori_loop(0, NPAIR, pair_body, 0)

        parts = [(0, head_rows)] + list(zip(tail_offs, wo_tail))
        for i, (lo, n) in enumerate(parts):
            wait_all(wo_v.at[pl.ds(lo, n)], sems.at[i])
            d = jnp.dot(o_s[:, lo:lo + n].astype(jnp.bfloat16), wo_v[lo:lo + n, :], preferred_element_type=jnp.float32)
            acc = d if i == 0 else acc_s[...] + d
            if i < len(parts) - 1:
                acc_s[...] = acc
        s_out = acc[0:1] + acc[1:2]
        out_ref[0] = (x + s_out * g[0:1]).astype(out_ref.dtype)

    def fn(A_x, A_k_cache, A_v_cache, A_wq, A_wo, B_x, B_w1, B_w3, B_w2):
        B, Sq, D = A_x.shape
        _, Hkv, Sk, Dh = A_k_cache.shape
        W = min(4096, max(256, Sk // 4))
        kt = jnp.swapaxes(A_k_cache, 2, 3).reshape(Hkv * Dh, Sk)
        vt = jnp.swapaxes(A_v_cache, 2, 3).reshape(Hkv * Dh, Sk)
        hbm = pl.BlockSpec(memory_space=pltpu.HBM)
        dt = A_x.dtype
        return pl.pallas_call(
            kernel,
            out_shape=jax.ShapeDtypeStruct((B, Sq, D), dt),
            in_specs=[hbm] * 8,
            out_specs=pl.BlockSpec(memory_space=pltpu.VMEM),
            scratch_shapes=[
                pltpu.VMEM((B, Sq, D), dt),
                pltpu.VMEM(A_wq.shape, dt),
                pltpu.VMEM(A_wo.shape, dt),
                pltpu.VMEM(B_w1.shape, dt),
                pltpu.VMEM(B_w3.shape, dt),
                pltpu.VMEM(B_w2.shape, dt),
                pltpu.VMEM((NBUF, PAIR, W), dt),
                pltpu.VMEM((NBUF, PAIR, W), dt),
                pltpu.VMEM((NPAIR, M, PAIR), jnp.float32),
                pltpu.VMEM((M, HQ * DH), jnp.float32),
                pltpu.VMEM((M, D), jnp.float32),
                pltpu.SemaphoreType.DMA((4,)),
            ],
            compiler_params=pltpu.CompilerParams(vmem_limit_bytes=110 * 1024 * 1024),
        )(A_x, kt, vt, A_wq, A_wo, B_w1, B_w3, B_w2)
    return fn


_impl = build(wq_slabs=10, wo_slabs=4, tail_p1=256)


@jax.jit
def pallas_recurrent_scan__sliding_block_cached__glu_gated_swiglu__decode_kernel(
    A_x: jax.Array,
    A_k_cache: jax.Array,
    A_v_cache: jax.Array,
    A_wq: jax.Array,
    A_wo: jax.Array,
    B_x: jax.Array,
    B_w1: jax.Array,
    B_w3: jax.Array,
    B_w2: jax.Array,
):
    return _impl(A_x, A_k_cache, A_v_cache, A_wq, A_wo, B_x, B_w1, B_w3, B_w2)
```

```python
import jax
import jax.numpy as jnp
from jax import lax
import jax.experimental.pallas as pl
import jax.experimental.pallas.tpu as pltpu

HQ, DH = 32, 192
PAIR = 2 * DH
NPAIR = HQ // 2
M = 8
TN = 2048
WQ_SLABS = 10
WO_SLABS = 4
WO_TAIL = (2048, 768, 256)
LN_EPS = 1e-5


def _silu(x):
    return x * jax.nn.sigmoid(x)


def _split(items, n):
    cuts = [len(items) * i // n for i in range(n + 1)]
    return [items[cuts[i]:cuts[i + 1]] for i in range(n)]


def _wo_plan(n_issue):
    head = HQ * DH - sum(WO_TAIL)
    parts, lo = [(0, head)], head
    for n in WO_TAIL:
        parts.append((lo, n))
        lo += n
    slab = head // WO_SLABS
    head_desc = [(s * slab + a, 24, 0) for a in range(0, slab, 24) for s in range(WO_SLABS)]
    tail_desc = [(r, 32, i) for i, (lo, n) in enumerate(parts) if i for r in range(lo, lo + n, 32)]
    last = len(parts) - 1
    desc = [d + (1 if d[2] == last else i % 2,) for i, d in enumerate(head_desc + tail_desc)]
    n_head = n_issue * head // (HQ * DH)
    groups = _split(desc[:len(head_desc)], n_head) + _split(desc[len(head_desc):], n_issue - n_head)
    assert all(g >= d[2] * (n_issue // 4) for g, group in enumerate(groups) for d in group)
    return parts, groups


def _kernel(x_hbm, kt_hbm, vt_hbm, wq_hbm, wo_hbm, w1_hbm, w3_hbm, w2_hbm, out_ref,
            x_v, wq_v, wo_v, w13_v, w2_v, kbuf, vbuf, q_s, o_s, acc_s, sems):
    D = x_v.shape[-1]
    F = w13_v.shape[-1]
    W = kbuf.shape[-1]
    win0 = kt_hbm.shape[-1] - W
    nblk = W // TN

    def aligned(i, n):
        return i if isinstance(i, int) else pl.multiple_of(i, n)

    def k_sem(slot):
        return sems.at[2 * slot]

    def v_sem(slot):
        return sems.at[2 * slot + 1]

    def wait_filled(buf, sem):
        pltpu.make_async_copy(buf, buf, sem).wait()

    def start_w(src, dst, sem, r0, rows, c0, cols, queue):
        pltpu.make_async_copy(src.at[pl.ds(r0, rows), pl.ds(c0, cols)],
                              dst.at[pl.ds(r0, rows), pl.ds(c0, cols)], sem).start(priority=queue)

    def start_kv(src, dst, sem, pair, slot, blk, rows=range(0, PAIR, 8)):
        for i, a in enumerate(rows):
            pltpu.make_async_copy(
                src.at[pl.ds(aligned(pair * PAIR + a, 8), 8), pl.ds(aligned(win0 + blk * TN, TN), TN)],
                dst.at[slot, pl.ds(aligned(a, 8), 8), pl.ds(aligned(blk * TN, TN), TN)],
                sem).start(priority=i % 2)

    wo_parts, wo_groups = _wo_plan(4 * nblk)

    def start_wo(group):
        for (r0, rows, part, queue) in wo_groups[group]:
            start_w(wo_hbm, wo_v, sems.at[part], r0, rows, 0, D, queue)

    x_cp = pltpu.make_async_copy(x_hbm, x_v, v_sem(1))
    x_cp.start()
    slab = D // WQ_SLABS
    wq_desc = [(r, c) for a in range(0, slab, 8) for c in range(0, HQ * DH, TN) for r in range(a, D, slab)]
    for i, (r, c) in enumerate(wq_desc):
        start_w(wq_hbm, wq_v, k_sem(1), r, 8, c, TN, (i + 1) % 2)
    x_cp.wait()
    ffn_desc = []
    for r, down in zip(range(0, D, 8), _split(list(range(0, F, 24)), D // 8)):
        ffn_desc += [(w1_hbm, w13_v.at[0], v_sem(1), r, 8, 0, F), (w3_hbm, w13_v.at[1], v_sem(1), r, 8, 0, F)]
        ffn_desc += [(w2_hbm, w2_v, sems.at[4], r2, 24, 0, D) for r2 in down]
    for i, d in enumerate(ffn_desc):
        start_w(*d, (i + 1) % 2)

    x = x_v[0].astype(jnp.float32)
    xc = x - jnp.mean(x, axis=-1, keepdims=True)
    var = jnp.mean(xc * xc, axis=-1, keepdims=True)
    xn = jnp.broadcast_to(xc / jnp.sqrt(var + LN_EPS), (M, D)).astype(jnp.bfloat16)

    row = lax.broadcasted_iota(jnp.int32, (M, PAIR), 0)
    col = lax.broadcasted_iota(jnp.int32, (M, PAIR), 1)
    own = ((row == 0) & (col < DH)) | ((row == 1) & (col >= DH))

    wait_filled(wq_v, k_sem(1))
    k0_rows = PAIR * nblk // NPAIR

    def q_body(p, carry):
        w = wq_v[:, pl.ds(pl.multiple_of(p * PAIR, 128), PAIR)]
        q_s[p] = jnp.where(own, jnp.dot(xn, w, preferred_element_type=jnp.float32), 0.0)
        a0 = lax.rem(p * k0_rows, PAIR)
        start_kv(kt_hbm, kbuf, k_sem(0), 0, 0, lax.div(p * k0_rows, PAIR),
                 [a0 + a for a in range(0, k0_rows, 8)])
        return carry

    lax.fori_loop(0, NPAIR, q_body, 0)

    for b in range(nblk):
        start_kv(vt_hbm, vbuf, v_sem(0), 0, 0, b)
    wait_filled(w13_v, v_sem(1))
    gate = jnp.dot(xn, w13_v[0], preferred_element_type=jnp.float32)
    up = jnp.dot(xn, w13_v[1], preferred_element_type=jnp.float32)
    h = (_silu(gate) * up).astype(jnp.bfloat16)
    for b in range(nblk):
        start_kv(kt_hbm, kbuf, k_sem(1), 1, 1, b)
    wait_filled(w2_v, sems.at[4])
    g = _silu(jnp.dot(h, w2_v[...], preferred_element_type=jnp.float32))
    for b in range(nblk):
        start_kv(vt_hbm, vbuf, v_sem(1), 1, 1, b)

    def pair_body(p, carry):
        slot = lax.rem(p, 2)

        def refill(src, dst, sem, phase, b):
            pl.when(p < NPAIR - 2)(lambda: start_kv(src, dst, sem, p + 2, slot, b))
            pl.when(p == NPAIR - 2)(lambda: start_wo(phase * nblk + b))
            pl.when(p == NPAIR - 1)(lambda: start_wo((2 + phase) * nblk + b))

        wait_filled(kbuf.at[slot], k_sem(slot))
        q = q_s[p].astype(jnp.bfloat16)
        s = []
        for b in range(nblk):
            s.append(jnp.dot(q, kbuf[slot, :, b * TN:(b + 1) * TN],
                             preferred_element_type=jnp.float32) * (DH ** -0.5))
            refill(kt_hbm, kbuf, k_sem(slot), 0, b)

        m = s[0]
        for sb in s[1:]:
            m = jnp.maximum(m, sb)
        m = jnp.max(m, axis=-1, keepdims=True)
        e = [jnp.exp(sb - m) for sb in s]
        denom = e[0]
        for eb in e[1:]:
            denom = denom + eb
        denom = jnp.sum(denom, axis=-1, keepdims=True)

        wait_filled(vbuf.at[slot], v_sem(slot))
        o = None
        for b in range(nblk):
            ob = lax.dot_general(e[b].astype(jnp.bfloat16), vbuf[slot, :, b * TN:(b + 1) * TN],
                                 (((1,), (1,)), ((), ())), preferred_element_type=jnp.float32)
            o = ob if o is None else o + ob
            refill(vt_hbm, vbuf, v_sem(slot), 1, b)

        o_s[:, pl.ds(pl.multiple_of(p * PAIR, 128), PAIR)] = jnp.where(own, o / denom, 0.0)
        return carry

    lax.fori_loop(0, NPAIR, pair_body, 0)

    for i, (lo, n) in enumerate(wo_parts):
        wait_filled(wo_v.at[pl.ds(lo, n)], sems.at[i])
        acc = jnp.dot(o_s[:, lo:lo + n].astype(jnp.bfloat16), wo_v[lo:lo + n, :],
                      preferred_element_type=jnp.float32)
        if i > 0:
            acc = acc_s[...] + acc
        if i < len(wo_parts) - 1:
            acc_s[...] = acc
    out_ref[0] = (x + (acc[0:1] + acc[1:2]) * g[0:1]).astype(out_ref.dtype)


@jax.jit
def pallas_recurrent_scan__sliding_block_cached__glu_gated_swiglu__decode_kernel(
    A_x: jax.Array,
    A_k_cache: jax.Array,
    A_v_cache: jax.Array,
    A_wq: jax.Array,
    A_wo: jax.Array,
    B_x: jax.Array,
    B_w1: jax.Array,
    B_w3: jax.Array,
    B_w2: jax.Array,
):
    del B_x
    B, Sq, D = A_x.shape
    _, Hkv, Sk, Dh = A_k_cache.shape
    W = min(4096, max(256, Sk // 4))
    assert (B, Sq, Hkv, Dh) == (1, 1, HQ, DH) and W % TN == 0 and Sk % TN == 0
    kt = jnp.swapaxes(A_k_cache, 2, 3).reshape(Hkv * Dh, Sk)
    vt = jnp.swapaxes(A_v_cache, 2, 3).reshape(Hkv * Dh, Sk)
    dt = A_x.dtype
    return pl.pallas_call(
        _kernel,
        out_shape=jax.ShapeDtypeStruct((B, Sq, D), dt),
        in_specs=[pl.BlockSpec(memory_space=pltpu.HBM)] * 8,
        out_specs=pl.BlockSpec(memory_space=pltpu.VMEM),
        scratch_shapes=[
            pltpu.VMEM((B, Sq, D), dt),
            pltpu.VMEM(A_wq.shape, dt),
            pltpu.VMEM(A_wo.shape, dt),
            pltpu.VMEM((2,) + B_w1.shape, dt),
            pltpu.VMEM(B_w2.shape, dt),
            pltpu.VMEM((2, PAIR, W), dt),
            pltpu.VMEM((2, PAIR, W), dt),
            pltpu.VMEM((NPAIR, M, PAIR), jnp.float32),
            pltpu.VMEM((M, HQ * DH), jnp.float32),
            pltpu.VMEM((M, D), jnp.float32),
            pltpu.SemaphoreType.DMA((5,)),
        ],
        compiler_params=pltpu.CompilerParams(vmem_limit_bytes=64 * 1024 * 1024),
    )(A_x, kt, vt, A_wq, A_wo, B_w1, B_w3, B_w2)
```
